```python
import os as _os
_os.environ.setdefault("JAX_PLATFORMS", "cpu")
import jax
import jax.numpy as jnp

def _softmax(x, axis=-1):
    return jax.nn.softmax(x, axis=axis)
def _gelu(x):
    return jax.nn.gelu(x, approximate=True)
def _silu(x):
    return jax.nn.silu(x)
def _sigmoid(x):
    return jax.nn.sigmoid(x)
def _layernorm(x, axis=-1, eps=1e-5):
    m = jnp.mean(x, axis=axis, keepdims=True)
    v = jnp.var(x, axis=axis, keepdims=True)
    return (x - m) / jnp.sqrt(v + eps)
def _scatter_add(tgt, idx, src, axis=0):
    return tgt.at[idx].add(src)
def _segment_sum(src, seg, n):
    return jax.ops.segment_sum(src, seg, n)
class _Rng:
    def __init__(self, key):
        self._k = key
    def _next(self):
        self._k, sub = jax.random.split(self._k)
        return sub
    def normal(self, shape):
        return jax.random.normal(self._next(), shape, dtype=jnp.bfloat16)
    def randint(self, lo, hi, shape):
        return jax.random.randint(self._next(), shape, lo, hi, dtype=jnp.int32)
    def uniform(self, shape, lo=0.0, hi=1.0):
        return jax.random.uniform(self._next(), shape, jnp.bfloat16, lo, hi)
    def permutation(self, n):
        return jax.random.permutation(self._next(), n)


kernel_name = 'interleave_layers__grouped_kv_mqa__sliding_block__prompt'

def setup_inputs():
    _rng = _Rng(jax.random.key(int.from_bytes(__import__("os").urandom(4), "little")))
    _w = (lambda a: (lambda t: t.astype(jnp.bfloat16) if jnp.issubdtype(t.dtype, jnp.floating) else t)(jnp.asarray(a)))
    def _A_setup():
        B, S, D, H = 1, 2048, 448, 16
        Dh = D // H
        return {
            "x": _w((lambda *s: _rng.normal(s) * 0.05)(B, S, D)),
            "wq": _w((lambda *s: _rng.normal(s) * 0.05)(D, H * Dh)),
            "wk": _w((lambda *s: _rng.normal(s) * 0.05)(D, Dh)),
            "wv": _w((lambda *s: _rng.normal(s) * 0.05)(D, Dh)),
            "wo": _w((lambda *s: _rng.normal(s) * 0.05)(H * Dh, D)),
        }
    _A_in = _A_setup()

    def _B_setup():
        B, S, D = 1, 2048, 448
        return {
            "x": _w((lambda *s: _rng.normal(s) * 0.05)(B, S, D)),
            "wqkv": _w((lambda *s: _rng.normal(s) * 0.05)(D, 3 * D)),
            "wo": _w((lambda *s: _rng.normal(s) * 0.05)(D, D)),
        }
    _B_in = _B_setup()

    return {
        "A_x": _A_in["x"],
        "A_wq": _A_in["wq"],
        "A_wk": _A_in["wk"],
        "A_wv": _A_in["wv"],
        "A_wo": _A_in["wo"],
        "B_x": _B_in["x"],
        "B_wqkv": _B_in["wqkv"],
        "B_wo": _B_in["wo"],
    }

def reference(A_x, A_wq, A_wk, A_wv, A_wo, B_x, B_wqkv, B_wo):
    def _A_ref(x, wq, wk, wv, wo):
        B, S, D = x.shape
        H = 16
        Dh = D // H
        q = (lambda x, *d: x.transpose(*d))((x @ wq).reshape(B, S, H, Dh), 0, 2, 1, 3)
        k = x @ wk
        v = x @ wv
        scores = jnp.einsum("bhqd,bkd->bhqk", q, k) * (Dh ** -0.5)
        p = _softmax(scores, axis=-1)
        o = jnp.einsum("bhqk,bkd->bhqd", p, v)
        return (lambda x, *d: x.transpose(*d))(o, 0, 2, 1, 3).reshape(B, S, H * Dh) @ wo

    def _B_ref(x, wqkv, wo):
        B, S, D = x.shape
        H = 16; Dh = D // H; W = 256
        qkv = (lambda x, *d: x.transpose(*d))((x @ wqkv).reshape(B, S, 3, H, Dh), 2, 0, 3, 1, 4)
        q, k, v = qkv[0], qkv[1], qkv[2]
        scores = jnp.einsum("bhqd,bhkd->bhqk", q, k) * (Dh ** -0.5)
        idx = jnp.arange(S)
        mask = (idx[:, None] - idx[None, :] >= 0) & (idx[:, None] - idx[None, :] < W)
        scores = jnp.where(mask[None, None], scores, -1e9)
        p = _softmax(scores, axis=-1)
        o = jnp.einsum("bhqk,bhkd->bhqd", p, v)
        return (lambda x, *d: x.transpose(*d))(o, 0, 2, 1, 3).reshape(B, S, D) @ wo

    x = A_x
    x = x + _A_ref(_layernorm(x, axis=-1), A_wq, A_wk, A_wv, A_wo)
    x = x + _B_ref(_layernorm(x, axis=-1), B_wqkv, B_wo)
    x = x + _A_ref(_layernorm(x, axis=-1), A_wq, A_wk, A_wv, A_wo)
    x = x + _B_ref(_layernorm(x, axis=-1), B_wqkv, B_wo)
    return x
```

```python
import functools

import jax
import jax.numpy as jnp
import numpy as np
from jax import lax
import jax.experimental.pallas as pl
import jax.experimental.pallas.tpu as pltpu

BF = jnp.bfloat16
F32 = jnp.float32
U32 = jnp.uint32

S = 2048
D = 448
H = 16
DH = D // H
HP = 32
HALF = D // 2
EPS = 1e-5
QSCALE = float(DH ** -0.5 * np.log2(np.e))

L_MIN = 2.0 ** -30
ACC_MAX = 2.0 ** 100

TC = 512
NCH = S // TC
TH = TC // 256

A_KEYS = 128
A_QUERIES = 512
A_HEADS = 2
A_SLOTS = 8
VPU_KEYS = 208
VPU_PERIOD = 43.6
B_LAG = 12
B_SLOTS = 24


def _dot(a, b):
    return lax.dot_general(a, b, (((1,), (0,)), ((), ())), preferred_element_type=F32)


def _words(ref, idx):
    return pltpu.bitcast(ref.bitcast(U32)[idx], BF)


def _tiles(ref, pre, c0, n):
    return jnp.concatenate([_words(ref, pre + (t,)) for t in range(c0 // 128, (c0 + n) // 128)], axis=1)


def _put_tiles(ref, pre, c0, val):
    for t in range(val.shape[1] // 128):
        ref[pre + (c0 // 128 + t,)] = val[:, 128 * t:128 * (t + 1)].astype(BF)


def _pad_head(rows, h, fill):
    r0 = 2 * DH * (h // 2) + (2 * DH - HP if h % 2 else 0)
    w = rows[r0:r0 + HP]
    if fill is None:
        return w
    sub = lax.broadcasted_iota(jnp.int32, (8, rows.shape[1]), 0)
    if h % 2 == 0:
        return jnp.concatenate([w[0:24], jnp.where(sub < 4, w[24:32], fill)], axis=0)
    return jnp.concatenate([jnp.where(sub >= 4, w[0:8], fill), w[8:32]], axis=0)


def _normalise(acc, odd):
    l = acc[0:1] if odd else acc[HP - 1:HP]
    o = acc * (1.0 / l)
    mag = jnp.max(jnp.abs(acc).reshape(HP // 8, 8, acc.shape[1]), axis=0)
    return o, jnp.where((mag <= ACC_MAX) & (l >= L_MIN), 0.0, 1.0)


def _put_weight(dst, top, bottom, r0=0):
    k = top.shape[1] // 2
    a11, a12, a21, a22 = top[:, :k], top[:, k:], bottom[:, :k], bottom[:, k:]
    for i, a in enumerate([a11 + a22, a21 + a22, a11, a22, a11 + a12, a21 - a11, a12 - a22]):
        for t in range(2):
            k1 = min(128 * (t + 1), k)
            dst[i, t, pl.ds(r0, a.shape[0]), pl.ds(0, k1 - 128 * t)] = a[:, 128 * t:k1].astype(BF)


def _matmul(w, k, rhs, done):
    def product(i, b):
        lhs = jnp.concatenate([_words(w, (i, 0)), _words(w, (i, 1, slice(None), slice(0, k - 128)))], axis=1)
        return _dot(lhs, b.astype(BF))

    b11, b12, b21, b22 = (functools.partial(rhs, *ij) for ij in ((0, 1), (0, 0), (1, 1), (1, 0)))
    m2 = product(1, b11())
    m5 = product(4, b22())
    m1 = product(0, b11() + b22())
    c11, c22 = m1 - m5, m1 - m2
    m3 = product(2, b12() - b22())
    done(0, 0, m3 + m5)
    c22 = c22 + m3
    done(1, 0, c22 + product(5, b11() + b12()))
    m4 = product(3, b21() - b11())
    done(1, 1, m2 + m4)
    c11 = c11 + m4
    done(0, 1, c11 + product(6, b21() + b22()))


class _Pacer:
    def __init__(self, scratch):
        self.scratch = scratch
        self.never = scratch[1] != 0.0
        self.clock = self.now = None

    def advance(self, cycle):
        while self.clock is not None and self.now + 2 <= cycle:
            self.clock, self.now = self.clock + 1.0, self.now + 2

    def mark(self, cycle, value):
        self.advance(cycle)
        if self.clock is None:
            self.clock, self.now = value, cycle
        else:
            self.clock, self.now = jnp.where(self.never, value, self.clock), self.now + 1

    def finish(self, cycle, result):
        self.advance(cycle)
        self.scratch[0] = jnp.zeros((8, 128), F32)
        return jnp.where(self.scratch[0] != 0.0, self.clock, result)


def _kernel(xT_hbm, wq_hbm, wkT_hbm, wvT_hbm, woa_hbm, wqkv_hbm, wob_hbm, out_hbm,
            x_io, wq_in, wkT_in, wvT_in, woa_in, wqkv_in, wob_in,
            WA, WOA, WB, WOB, QT, QF, KA, KF, KBC, VA, KS, VB, OT, BAD, PACE, ZERO, sems,
            X, VP, PA, PB):

    def put_x(c, i, j, x):
        for t in range(TH):
            X[c][ZERO[0] + TH * j + t, pl.ds(i * HALF, HALF), :] = x[:, 128 * t:128 * (t + 1)]

    def get_x(c, i, j):
        return jnp.concatenate([X[c][TH * j + t, pl.ds(i * HALF, HALF), :] for t in range(TH)], axis=1)

    def layernorm(c, pacer=None, now=0):
        def total(v):
            acc = [v[r:r + 8] for r in range(0, 32, 8)]
            for i in range(4, D // 8):
                acc[i % 4] = acc[i % 4] + v[8 * i:8 * i + 8]
            return jnp.sum(functools.reduce(jnp.add, acc), axis=0, keepdims=True) * (1.0 / D)

        coef, calls = [], [0]
        for t in range(TC // 128):
            x = X[c][t]
            mean = total(x)
            centred = x - mean
            inv = lax.rsqrt(total(centred * centred) + EPS)
            coef.append((inv, mean * inv))
            if pacer is not None:
                pacer.mark(now + 500 + 280 * t, jnp.broadcast_to(inv, (8, 128)))

        def quadrant(i, j):
            calls[0] += 1
            base = ZERO[calls[0]]
            return jnp.concatenate(
                [X[c][base + TH * j + t, pl.ds(i * HALF, HALF), :] * coef[TH * j + t][0] - coef[TH * j + t][1]
                 for t in range(TH)], axis=1)

        return quadrant

    def project_a(c, xn):
        def done(i, j, r):
            c0 = c * TC + j * (TC // 2)
            cols = pl.ds(c0, TC // 2)
            q = r[HP:] * QSCALE
            for h in range(H // 2):
                qh = _pad_head(q, h, None)
                _put_tiles(QT, (h + i * (H // 2),), c0, qh)
                QF[h + i * (H // 2), :, cols] = qh
            even = r[0:HP]
            odd = jnp.concatenate([even[DH:HP], even[0:DH]], axis=0)
            sub = lax.broadcasted_iota(jnp.int32, even.shape, 0)
            spare = 0.0 if i == 0 else 1.0
            even, odd = jnp.where(sub < DH, even, spare), jnp.where(sub >= HP - DH, odd, spare)
            if i == 0:
                KA[0, cols, :] = even.astype(BF).T
                KA[1, cols, :] = odd.astype(BF).T
                if (c, j) == (0, 0):
                    KF[...] = even[:, 0:256]
                if (c, j) == (1, 0):
                    kt = KF[...].T[0:VPU_KEYS]
                    for d in range(DH):
                        KBC[d] = jnp.broadcast_to(kt[:, d:d + 1], (VPU_KEYS, 128))
            else:
                _put_tiles(VA, (0,), c0, even)
                _put_tiles(VA, (1,), c0, odd)

        _matmul(WA, HALF, xn, done)

    def project_b(c, xn, k_prev):
        def done(i, j, r):
            c0 = c * TC + j * (TC // 2)
            k, q, v = r[0:HALF], r[HALF:2 * HALF] * QSCALE, r[2 * HALF:3 * HALF]
            kp = jnp.concatenate([_pad_head(k, h, 0.0) for h in range(H // 2)], axis=0)
            kt = pltpu.bitcast(kp.astype(BF).T, U32)
            ext = jnp.concatenate([k_prev[i], kt], axis=0)
            n = kt.shape[0]
            k_prev[i] = kt[n - 48:]
            group = lax.broadcasted_iota(jnp.int32, (n, 128), 1) // HP
            for h0 in range(0, H // 2, 4):
                four = ext[:, HP * h0:HP * (h0 + 4)]
                rolled = [four] + [pltpu.roll(four, HP * s, 1) for s in (1, 2, 3)]
                for h in range(4):
                    w = rolled[-h % 4][0:n]
                    for g in (1, 2, 3):
                        w = jnp.where(group == g, rolled[(g - h) % 4][16 * g:16 * g + n], w)
                    KS[h0 + h + i * (H // 2), pl.ds(c0 // 2, n), :] = w
            for h in range(H // 2):
                _put_tiles(QT, (h + i * (H // 2),), c0, _pad_head(q, h, None))
                _put_tiles(VB, (h + i * (H // 2),), c0, _pad_head(v, h, 1.0))

        _matmul(WB, HALF, xn, done)

    def out_proj(wo, c, done):
        def quadrant(i, j):
            return OT[pl.ds(i * 256, 256), pl.ds(c * TC + j * (TC // 2), TC // 2)]

        _matmul(wo, 256, quadrant, lambda i, j, r: done(c, i, j, get_x(c, i, j) + r))

    def between_layers(wo, project, cycles=None):
        out_proj(wo, 0, put_x)
        now, xn = 7 * HALF, {}
        pacer = _Pacer(PACE) if cycles else None
        for c in range(NCH):
            if c not in xn:
                xn[c] = layernorm(c, pacer, now)
            if c + 1 < NCH:
                out_proj(wo, c + 1, put_x)
                now += 7 * HALF
            if c + 2 == NCH:
                xn[c + 1] = layernorm(c + 1, pacer, now)
            project(c, xn[c])
            now += cycles or 0
        if cycles:
            PACE[2] = pacer.finish(now + 200, jnp.zeros((8, 128), F32))

    def put_wo(src, dst):
        w = src[...].astype(F32)
        wt = jnp.concatenate([_pad_head(w, h, 0.0) for h in range(H)], axis=0).astype(BF).T.astype(F32)
        _put_weight(dst, wt[:HALF], wt[HALF:])

    def attention_a():
        first = -(-VPU_KEYS // A_KEYS) * A_KEYS
        ranges = [(k0, k0 + A_KEYS) for k0 in range(first, S, A_KEYS)] + [(VPU_KEYS, first)]
        last = len(ranges) - 1
        n_q, tq = S // A_QUERIES, A_QUERIES // 128

        def vpu_scores(h, odd, t, r):
            acc = None
            for d in range(DH):
                q = QF[h, pl.ds(d + 4 * odd, 1), pl.ds(t * 128, 128)]
                term = KBC[d, pl.ds(r, 16), :] * q
                acc = term if acc is None else acc + term
            return acc

        def body(it, carry):
            zero = ZERO[0]
            pacer = _Pacer(PACE)

            def vpu_probs():
                blocks = [(u, t, r) for u in range(A_HEADS) for t in range(S // 128) for r in range(0, VPU_KEYS, 16)]
                for j, (u, t, r) in enumerate(blocks):
                    vp = VP[u * n_q + t // tq]
                    p = jnp.exp2(vpu_scores(A_HEADS * it + u, u % 2, t, r))
                    vp[zero + t % tq, pl.ds(r, 16), :] = p.astype(BF)
                    pacer.mark(j * VPU_PERIOD, vp.bitcast(F32)[tq, pl.ds(0, 8), :])
                    pacer.advance((j + 1) * VPU_PERIOD)

            items = [(u, n, j) for u in range(A_HEADS) for n in range(last) for j in range(n_q)]
            n_plain = len(items)
            items += [(u, last, j) for u in range(A_HEADS) for j in range(n_q)]
            accs, bad = {}, None
            for i in range(len(items) + n_q):
                if i == n_plain:
                    vpu_probs()
                if i < len(items):
                    u, n, j = items[i]
                    k0, k1 = ranges[n]
                    k = _words(KA, (u % 2, pl.ds(k0 // 2, (k1 - k0) // 2)))
                    p = jnp.exp2(_dot(k, _tiles(QT, (A_HEADS * it + u,), j * A_QUERIES, A_QUERIES)))
                    for t in range(tq):
                        PA[i % A_SLOTS][zero + t, pl.ds(0, k1 - k0), :] = p[:, 128 * t:128 * (t + 1)].astype(BF)
                if i >= n_q:
                    u, n, j = items[i - n_q]
                    k0, k1 = ranges[n]
                    slot = PA[(i - n_q) % A_SLOTS]
                    p = jnp.concatenate([_words(slot, (t, pl.ds(0, (k1 - k0) // 2))) for t in range(tq)], axis=1)
                    if n == last:
                        p = jnp.concatenate([_tiles(VP[u * n_q + j], (), 0, A_QUERIES), p], axis=0)
                        k0 = 0
                    o = _dot(_tiles(VA, (u % 2,), k0, k1 - k0), p)
                    accs[u, j] = o if n == 0 else accs[u, j] + o
                    if n == last:
                        o, b = _normalise(accs.pop((u, j)), u % 2)
                        rows = pl.ds(pl.multiple_of((A_HEADS * it + u) * HP, HP), HP)
                        OT[rows, pl.ds(j * A_QUERIES, A_QUERIES)] = o
                        b = functools.reduce(jnp.maximum, [b[:, 128 * t:128 * (t + 1)] for t in range(tq)])
                        bad = b if bad is None else jnp.maximum(bad, b)
            bad = pacer.finish(pacer.now + 600, bad)
            BAD[...] = jnp.maximum(BAD[...], bad)
            return carry

        lax.fori_loop(0, H // A_HEADS, body, 0)

    def attention_a_shifted():
        def body(it, carry):
            pair, t = it // (S // 128), it % (S // 128)
            for odd in range(2):
                s = _dot(KA[odd], QT[2 * pair + odd, t])
                p = jnp.exp2(s - jnp.max(s, axis=0, keepdims=True)).astype(BF)
                o, _ = _normalise(_dot(_tiles(VA, (odd,), 0, S), p), odd)
                OT[pl.ds(pl.multiple_of((2 * pair + odd) * HP, HP), HP), pl.ds(pl.multiple_of(t * 128, 128), 128)] = o
            return carry

        lax.fori_loop(0, (H // 2) * (S // 128), body, 0)

    def window_probs(h, i, b0, shifted):
        row = lax.broadcasted_iota(jnp.int32, (32, 128), 0)
        lane = lax.broadcasted_iota(jnp.int32, (32, 128), 1)
        q = QT.bitcast(U32)[h, i]
        w = jnp.concatenate([jnp.where(lane[0:16] // 32 == g, q, jnp.uint32(0)) for g in range(4)], axis=0)
        k0 = 64 * i - 80 + 16 * b0
        if not isinstance(k0, int):
            k0 = pl.multiple_of(k0, 16)
        s = _dot(pltpu.bitcast(KS[h, pl.ds(k0, 16 * (9 - b0)), :], BF), pltpu.bitcast(w, BF))
        e = {b: s[32 * (b - b0):32 * (b - b0 + 1)] for b in range(b0, 9)}
        masked = -jnp.inf if shifted else 0.0
        if not shifted:
            e = {b: jnp.exp2(v) for b, v in e.items()}
        if b0 == 0:
            e[0] = jnp.where(row > lane % 32, e[0], masked)
        e[8] = jnp.where(row <= lane % 32, e[8], masked)
        if shifted:
            for b in range(b0, b0 + 3 if b0 else b0):
                e[b] = jnp.where(lane // 32 >= 3 - (b - b0), e[b], masked)
            m = jnp.max(functools.reduce(jnp.maximum, e.values()), axis=0, keepdims=True)
            e = {b: jnp.exp2(v - m) for b, v in e.items()}

        def pick(mask, a, b):
            if a is None and b is None:
                return None
            return jnp.where(mask, 0.0 if a is None else a, 0.0 if b is None else b)

        f = {b: pick((lane // 32) % 2 == 1, e.get(b - 1), e.get(b)) for b in range(10)}
        start = {5: 8, 1: 4, 0: 0}[b0]
        p = [pick(lane >= 64, f.get(b - 2), f.get(b)) for b in range(start, 12)]
        return jnp.concatenate(p, axis=0).astype(BF)

    def window_output(h, odd, i, p):
        v = jnp.concatenate([_words(VB, (h, i - t)) for t in reversed(range(p.shape[0] // 128))], axis=1)
        o, bad = _normalise(_dot(v, p), odd)
        r0 = h * HP if isinstance(h, int) else pl.multiple_of(h * HP, HP)
        q0 = 128 * i if isinstance(i, int) else pl.multiple_of(128 * i, 128)
        OT[pl.ds(r0, HP), pl.ds(q0, 128)] = o
        return bad

    def attention_b():
        @pl.when(ZERO[15] == 0)
        def _():
            items = [(i, h) for i in range(S // 128) for h in range(H)]
            bad = None
            for n in range(len(items) + B_LAG):
                if n < len(items):
                    i, h = items[n]
                    p = window_probs(h, i, max(0, 5 - 4 * i), False)
                    PB[n % B_SLOTS][ZERO[0], pl.ds(0, p.shape[0]), :] = p
                if n >= B_LAG:
                    i, h = items[n - B_LAG]
                    p = _words(PB[(n - B_LAG) % B_SLOTS], (0, pl.ds(0, 64 * min(i + 1, 3))))
                    b = window_output(h, h % 2, i, p)
                    bad = b if bad is None else jnp.maximum(bad, b)
            BAD[...] = jnp.maximum(BAD[...], bad)

    def attention_b_shifted():
        def body(pair, carry):
            for odd in range(2):
                h = 2 * pair + odd
                window_output(h, odd, 0, window_probs(h, 0, 5, True))
                window_output(h, odd, 1, window_probs(h, 1, 1, True))

                def inner(i, c):
                    window_output(h, odd, i, window_probs(h, i, 0, True))
                    return c

                lax.fori_loop(2, S // 128, inner, 0)
            return carry

        lax.fori_loop(0, H // 2, body, 0)

    def guarded(plain, shifted):
        BAD[...] = jnp.zeros(BAD.shape, F32)
        plain()

        @pl.when(jnp.max(BAD[...]) > 0.0)
        def _():
            shifted()

    x_copies = [pltpu.make_async_copy(xT_hbm.at[:, pl.ds(c * TC, TC)], x_io.at[:, pl.ds(c * TC, TC)], sems.at[c])
                for c in range(NCH)]
    w_copies = [pltpu.make_async_copy(src, dst, sems.at[NCH + i]) for i, (src, dst) in enumerate([
        (wq_hbm, wq_in), (wkT_hbm, wkT_in), (wvT_hbm, wvT_in),
        (woa_hbm, woa_in), (wqkv_hbm, wqkv_in), (wob_hbm, wob_in)])]
    first_copies = w_copies[:1] + x_copies[:1] + w_copies[1:3]
    for cp in first_copies + x_copies[1:]:
        cp.start()
    for i in range(16):
        ZERO[i] = 0
    PACE[ZERO[0] + 1] = jnp.zeros((8, 128), F32)
    for vp in VP:
        vp[A_QUERIES // 128, pl.ds(0, 16), :] = jnp.zeros((16, 128), BF)

    def first_projection(c):
        for j in range(2):
            for i in range(2):
                put_x(c, i, j, x_io[pl.ds(i * HALF, HALF), pl.ds(c * TC + j * (TC // 2), TC // 2)].astype(F32))
        project_a(c, layernorm(c))

    for cp in first_copies:
        cp.wait()
    wt = wq_in[...].T.astype(F32)
    pad = jnp.zeros((HP - DH, D), F32)
    _put_weight(WA, jnp.concatenate([wkT_in[...].astype(F32), pad, wt[:HALF]], axis=0),
                jnp.concatenate([wvT_in[...].astype(F32), pad, wt[HALF:]], axis=0))
    first_projection(0)
    for cp in x_copies[1:]:
        cp.wait()
    for cp in w_copies[3:]:
        cp.start()
    for c in range(1, NCH):
        first_projection(c)

    for layer_pair in range(2):
        guarded(attention_a, attention_a_shifted)
        if layer_pair == 0:
            for cp in w_copies[3:]:
                cp.wait()
            put_wo(woa_in, WOA)
            wt = wqkv_in[...].T.astype(F32)
            for j, pos in enumerate((1, 0, 2)):
                _put_weight(WB, wt[j * D:j * D + HALF], wt[j * D + HALF:(j + 1) * D], pos * HALF)
        k_prev = [jnp.zeros((48, H * HP // 2), U32)] * 2
        between_layers(WOA, functools.partial(project_b, k_prev=k_prev))
        if layer_pair == 0:
            put_wo(wob_in, WOB)
        guarded(attention_b, attention_b_shifted)
        if layer_pair == 0:
            between_layers(WOB, project_a, 7 * (HALF + HP))

    outs = []

    def send(idx):
        outs.append(pltpu.make_async_copy(x_io.at[idx], out_hbm.at[idx], sems.at[len(outs)]))
        outs[-1].start()

    def emit(c, i, j, x):
        idx = (pl.ds(i * HALF, HALF), pl.ds(c * TC + j * (TC // 2), TC // 2))
        x_io[idx] = x.astype(BF)
        if c == NCH - 1:
            send(idx)

    for c in range(NCH):
        out_proj(WOB, c, emit)
        if c < NCH - 1:
            send((slice(None), pl.ds(c * TC, TC)))
    for cp in outs:
        cp.wait()


@jax.jit
def pallas_interleave_layers__grouped_kv_mqa__sliding_block__prompt_kernel(
    A_x: jax.Array,
    A_wq: jax.Array,
    A_wk: jax.Array,
    A_wv: jax.Array,
    A_wo: jax.Array,
    B_x: jax.Array,
    B_wqkv: jax.Array,
    B_wo: jax.Array,
):
    del B_x

    def weight(n):
        return pltpu.VMEM((7, 2, n, 128), BF)

    hbm = pl.BlockSpec(memory_space=pl.ANY)
    tq = A_QUERIES // 128
    out_t = pl.pallas_call(
        _kernel,
        out_shape=jax.ShapeDtypeStruct((D, S), BF),
        in_specs=[hbm] * 7,
        out_specs=hbm,
        scratch_shapes=[
            pltpu.VMEM((D, S), BF),
            pltpu.VMEM((D, D), BF), pltpu.VMEM((DH, D), BF), pltpu.VMEM((DH, D), BF),
            pltpu.VMEM((D, D), BF), pltpu.VMEM((D, 3 * D), BF), pltpu.VMEM((D, D), BF),
            weight(HALF + HP), weight(HALF), weight(3 * HALF), weight(HALF),
            pltpu.VMEM((H, S // 128, HP, 128), BF),
            pltpu.VMEM((H, HP, S), F32),
            pltpu.VMEM((2, S, HP), BF),
            pltpu.VMEM((HP, 256), F32),
            pltpu.VMEM((DH, VPU_KEYS, 128), F32),
            pltpu.VMEM((2, S // 128, HP, 128), BF),
            pltpu.VMEM((H, S // 2, 128), U32),
            pltpu.VMEM((H, S // 128, HP, 128), BF),
            pltpu.VMEM((H * HP, S), F32),
            pltpu.VMEM((8, 128), F32),
            pltpu.VMEM((3, 8, 128), F32),
            pltpu.SMEM((16,), jnp.int32),
            pltpu.SemaphoreType.DMA((16,)),
            [pltpu.VMEM((TC // 128, D, 128), F32)] * NCH,
            [pltpu.VMEM((tq + 1, VPU_KEYS, 128), BF)] * (A_HEADS * (S // A_QUERIES)),
            [pltpu.VMEM((tq, A_KEYS, 128), BF)] * A_SLOTS,
            [pltpu.VMEM((1, 384, 128), BF)] * B_SLOTS,
        ],
        compiler_params=pltpu.CompilerParams(vmem_limit_bytes=100 * 1024 * 1024),
        name="interleaved_attention",
    )(A_x.reshape(S, D).T, A_wq, A_wk.T, A_wv.T, A_wo, B_wqkv, B_wo)
    return out_t.T.reshape(1, S, D)
```

```python
import functools

import jax
import jax.numpy as jnp
import numpy as np
from jax import lax
import jax.experimental.pallas as pl
import jax.experimental.pallas.tpu as pltpu

BF = jnp.bfloat16
F32 = jnp.float32
U32 = jnp.uint32

S = 2048
D = 448
H = 16
DH = D // H
HP = 32
HALF = D // 2
EPS = 1e-5
QSCALE = float(DH ** -0.5 * np.log2(np.e))

L_MIN = 2.0 ** -30
ACC_MAX = 2.0 ** 100

TC = 512
NCH = S // TC

A_KEYS = 128
A_QUERIES = 512
A_HEADS = 2
A_SLOTS = 8
VPU_KEYS = 208
VPU_PERIOD = 43.6
B_LAG = 12
B_SLOTS = 24


def _dot(a, b):
    return lax.dot_general(a, b, (((1,), (0,)), ((), ())), preferred_element_type=F32)


def _words(ref, idx):
    return pltpu.bitcast(ref.bitcast(U32)[idx], BF)


def _tiles(ref, pre, c0, n):
    return jnp.concatenate([_words(ref, pre + (t,)) for t in range(c0 // 128, (c0 + n) // 128)], axis=1)


def _put_tiles(ref, pre, c0, val):
    for t in range(val.shape[1] // 128):
        ref[pre + (c0 // 128 + t,)] = val[:, 128 * t:128 * (t + 1)].astype(BF)


def _pad_head(rows, h, fill):
    r0 = 2 * DH * (h // 2) + (2 * DH - HP if h % 2 else 0)
    w = rows[r0:r0 + HP]
    if fill is None:
        return w
    sub = lax.broadcasted_iota(jnp.int32, (8, rows.shape[1]), 0)
    if h % 2 == 0:
        return jnp.concatenate([w[0:24], jnp.where(sub < 4, w[24:32], fill)], axis=0)
    return jnp.concatenate([jnp.where(sub >= 4, w[0:8], fill), w[8:32]], axis=0)


def _normalise(acc, odd):
    l = acc[0:1] if odd else acc[HP - 1:HP]
    o = acc * (1.0 / l)
    mag = jnp.max(jnp.abs(acc).reshape(HP // 8, 8, acc.shape[1]), axis=0)
    return o, jnp.where((mag <= ACC_MAX) & (l >= L_MIN), 0.0, 1.0)


def _put_weight(dst, top, bottom, r0=0):
    k = top.shape[1] // 2
    a11, a12, a21, a22 = top[:, :k], top[:, k:], bottom[:, :k], bottom[:, k:]
    for i, a in enumerate([a11 + a22, a21 + a22, a11, a22, a11 + a12, a21 - a11, a12 - a22]):
        for t in range(2):
            k1 = min(128 * (t + 1), k)
            dst[i, t, pl.ds(r0, a.shape[0]), pl.ds(0, k1 - 128 * t)] = a[:, 128 * t:k1].astype(BF)


def _matmul(w, k, rhs, done):
    def product(i, b):
        lhs = jnp.concatenate([_words(w, (i, 0)), _words(w, (i, 1, slice(None), slice(0, k - 128)))], axis=1)
        return _dot(lhs, b.astype(BF))

    b11, b12, b21, b22 = (0, 1), (0, 0), (1, 1), (1, 0)
    m2 = product(1, rhs(b11))
    m5 = product(4, rhs(b22))
    m1 = product(0, rhs(b11, b22))
    c11, c22 = m1 - m5, m1 - m2
    m3 = product(2, rhs(b12, b22, True))
    done(0, 0, m3 + m5)
    c22 = c22 + m3
    done(1, 0, c22 + product(5, rhs(b11, b12)))
    m4 = product(3, rhs(b21, b11, True))
    done(1, 1, m2 + m4)
    c11 = c11 + m4
    done(0, 1, c11 + product(6, rhs(b21, b22)))


class _Pacer:
    def __init__(self, scratch):
        self.scratch = scratch
        self.never = scratch[1] != 0.0
        self.clock = self.now = None

    def advance(self, cycle):
        while self.clock is not None and self.now + 2 <= cycle:
            self.clock, self.now = self.clock + 1.0, self.now + 2

    def mark(self, cycle, value):
        self.advance(cycle)
        if self.clock is None:
            self.clock, self.now = value, cycle
        else:
            self.clock, self.now = jnp.where(self.never, value, self.clock), self.now + 1

    def finish(self, cycle, result):
        self.advance(cycle)
        self.scratch[0] = jnp.zeros((8, 128), F32)
        return jnp.where(self.scratch[0] != 0.0, self.clock, result)


def _kernel(xT_hbm, wq_hbm, wkT_hbm, wvT_hbm, woa_hbm, wqkv_hbm, wob_hbm, out_hbm,
            x_io, wq_in, wkT_in, wvT_in, woa_in, wqkv_in, wob_in,
            WA, WOA, WB, WOB, QT, QF, KA, KF, KBC, VA, KS, VB, OT, BAD, PACE, ZERO, sems,
            X, VP, PA, PB):

    def half_tiles(chunk, j):
        n = len(chunk) // 2
        return chunk[j * n:(j + 1) * n]

    def x_tile(base, t, i):
        return X[t // 4], (base + t % 4, pl.ds(i * HALF, HALF))

    def put_x(chunk, i, j, x):
        for n, t in enumerate(half_tiles(chunk, j)):
            ref, idx = x_tile(ZERO[0], t, i)
            ref[idx] = x[:, 128 * n:128 * (n + 1)]

    def get_x(base, t, i):
        ref, idx = x_tile(base, t, i)
        return ref[idx]

    def layernorm(chunk, pacer=None, now=0):
        def mean_of(v):
            acc = [v[r:r + 8] for r in range(0, 32, 8)]
            for i in range(4, D // 8):
                acc[i % 4] = acc[i % 4] + v[8 * i:8 * i + 8]
            return jnp.sum(functools.reduce(jnp.add, acc), axis=0, keepdims=True) * (1.0 / D)

        coef, calls = {}, [0]
        for n, t in enumerate(chunk):
            x = X[t // 4][t % 4]
            mean = mean_of(x)
            centred = x - mean
            inv = lax.rsqrt(mean_of(centred * centred) + EPS)
            coef[t] = (inv, mean * inv)
            if pacer is not None:
                pacer.mark(now + 300 + 200 * n, jnp.broadcast_to(inv, (8, 128)))

        def quadrant(p, q=None, minus=False):
            calls[0] += 1
            base, out = ZERO[calls[0]], []
            for t, u in zip(half_tiles(chunk, p[1]), half_tiles(chunk, (q or p)[1])):
                if q is None:
                    out.append(get_x(base, t, p[0]) * coef[t][0] - coef[t][1])
                elif minus:
                    out.append((get_x(base, t, p[0]) - get_x(base, u, q[0])) * coef[t][0])
                else:
                    out.append(get_x(base, t, p[0]) * coef[t][0] + get_x(base, u, q[0]) * coef[u][0]
                               - (coef[t][1] + coef[u][1]))
            return jnp.concatenate(out, axis=1)

        return quadrant

    def project_a(chunk, xn):
        def done(i, j, r):
            c0 = 128 * half_tiles(chunk, j)[0]
            cols = pl.ds(c0, r.shape[1])
            q = r[HP:]
            for h in range(H // 2):
                qh = _pad_head(q, h, None)
                _put_tiles(QT, (h + i * (H // 2),), c0, qh)
                QF[h + i * (H // 2), :, cols] = qh
            even = r[0:HP]
            odd = jnp.concatenate([even[DH:HP], even[0:DH]], axis=0)
            sub = lax.broadcasted_iota(jnp.int32, even.shape, 0)
            spare = 0.0 if i == 0 else 1.0
            even, odd = jnp.where(sub < DH, even, spare), jnp.where(sub >= HP - DH, odd, spare)
            if i == 0:
                KA[0, cols, :] = even.astype(BF).T
                KA[1, cols, :] = odd.astype(BF).T
                if c0 == 0:
                    KF[...] = even[:, 0:256]
                if c0 == TC:
                    kt = KF[...].T[0:VPU_KEYS]
                    for d in range(DH):
                        KBC[pl.ds(d * VPU_KEYS, VPU_KEYS), :] = jnp.broadcast_to(kt[:, d:d + 1], (VPU_KEYS, 128))
            else:
                _put_tiles(VA, (0,), c0, even)
                _put_tiles(VA, (1,), c0, odd)

        _matmul(WA, HALF, xn, done)

    def project_b(chunk, xn, k_prev):
        def done(i, j, r):
            c0 = 128 * half_tiles(chunk, j)[0]
            k, q, v = r[0:HALF], r[HALF:2 * HALF], r[2 * HALF:3 * HALF]
            kp = jnp.concatenate([_pad_head(k, h, 0.0) for h in range(H // 2)], axis=0)
            kt = pltpu.bitcast(kp.astype(BF).T, U32)
            ext = jnp.concatenate([k_prev[i], kt], axis=0)
            n = kt.shape[0]
            k_prev[i] = kt[n - 48:]
            group = lax.broadcasted_iota(jnp.int32, (n, 128), 1) // HP
            for h0 in range(0, H // 2, 4):
                four = ext[:, HP * h0:HP * (h0 + 4)]
                rolled = [four] + [pltpu.roll(four, HP * s, 1) for s in (1, 2, 3)]
                for h in range(4):
                    w = rolled[-h % 4][0:n]
                    for g in (1, 2, 3):
                        w = jnp.where(group == g, rolled[(g - h) % 4][16 * g:16 * g + n], w)
                    KS[h0 + h + i * (H // 2), pl.ds(c0 // 2, n), :] = w
            for h in range(H // 2):
                _put_tiles(QT, (h + i * (H // 2),), c0, _pad_head(q, h, None))
                _put_tiles(VB, (h + i * (H // 2),), c0, _pad_head(v, h, 1.0))

        _matmul(WB, HALF, xn, done)

    def out_proj(wo, chunk, done):
        def load(i, j):
            tiles = half_tiles(chunk, j)
            return OT[pl.ds(i * 256, 256), pl.ds(128 * tiles[0], 128 * len(tiles))]

        def quadrant(p, q=None, minus=False):
            return load(*p) if q is None else load(*p) - load(*q) if minus else load(*p) + load(*q)

        def add_residual(i, j, r):
            done(chunk, i, j, jnp.concatenate([get_x(0, t, i) for t in half_tiles(chunk, j)], axis=1) + r)

        _matmul(wo, 256, quadrant, add_residual)

    def chunks(tokens):
        return [range(t, t + tokens // 128) for t in range(0, S // 128, tokens // 128)]

    def between_layers(wo, project, tokens, cycles=None):
        parts = chunks(tokens)
        out_proj(wo, parts[0], put_x)
        now, xn = 7 * HALF, {}
        pacer = _Pacer(PACE) if cycles else None
        for c, chunk in enumerate(parts):
            if c not in xn:
                xn[c] = layernorm(chunk, pacer, now)
            if c + 1 < len(parts):
                out_proj(wo, parts[c + 1], put_x)
                now += 7 * HALF
            if c + 2 == len(parts):
                xn[c + 1] = layernorm(parts[c + 1], pacer, now)
            project(chunk, xn[c])
            now += cycles or 0
        if cycles:
            PACE[2] = pacer.finish(now + 200, jnp.zeros((8, 128), F32))

    def put_wo(src, dst):
        w = src[...].astype(F32)
        wt = jnp.concatenate([_pad_head(w, h, 0.0) for h in range(H)], axis=0).astype(BF).T.astype(F32)
        _put_weight(dst, wt[:HALF], wt[HALF:])

    def attention_a():
        first = -(-VPU_KEYS // A_KEYS) * A_KEYS
        ranges = [(k0, k0 + A_KEYS) for k0 in range(first, S, A_KEYS)] + [(VPU_KEYS, first)]
        last = len(ranges) - 1
        n_q, tq = S // A_QUERIES, A_QUERIES // 128

        def body(it, carry):
            zero = ZERO[0]
            pacer = _Pacer(PACE)

            def vpu_probs():
                j = 0
                for u in range(A_HEADS):
                    qf = QF.at[A_HEADS * it + u]
                    for t in range(S // 128):
                        vp, q = VP[u * n_q + t // tq], {}
                        for r in range(0, VPU_KEYS, 16):
                            s = None
                            for d in range(DH):
                                if d not in q:
                                    row = qf[pl.ds(d + 4 * (u % 2), 1), pl.ds(t * 128, 128)]
                                    q[d] = jnp.broadcast_to(row, (16, 128))
                                term = KBC[pl.ds(d * VPU_KEYS + r, 16), :] * q[d]
                                s = term if s is None else s + term
                            vp[zero + t % tq, pl.ds(r, 16), :] = jnp.exp2(s).astype(BF)
                            pacer.mark(j * VPU_PERIOD, vp.bitcast(F32)[tq, pl.ds(0, 8), :])
                            j += 1
                            pacer.advance(j * VPU_PERIOD)

            items = [(u, n, j) for u in range(A_HEADS) for n in range(last) for j in range(n_q)]
            n_plain = len(items)
            items += [(u, last, j) for u in range(A_HEADS) for j in range(n_q)]
            accs, bad = {}, None
            for i in range(len(items) + n_q):
                if i == n_plain:
                    vpu_probs()
                if i < len(items):
                    u, n, j = items[i]
                    k0, k1 = ranges[n]
                    k = _words(KA, (u % 2, pl.ds(k0 // 2, (k1 - k0) // 2)))
                    p = jnp.exp2(_dot(k, _tiles(QT, (A_HEADS * it + u,), j * A_QUERIES, A_QUERIES)))
                    for t in range(tq):
                        PA[i % A_SLOTS][zero + t, pl.ds(0, k1 - k0), :] = p[:, 128 * t:128 * (t + 1)].astype(BF)
                if i >= n_q:
                    u, n, j = items[i - n_q]
                    k0, k1 = ranges[n]
                    slot = PA[(i - n_q) % A_SLOTS]
                    p = jnp.concatenate([_words(slot, (t, pl.ds(0, (k1 - k0) // 2))) for t in range(tq)], axis=1)
                    if n == last:
                        p = jnp.concatenate([_tiles(VP[u * n_q + j], (), 0, A_QUERIES), p], axis=0)
                        k0 = 0
                    o = _dot(_tiles(VA, (u % 2,), k0, k1 - k0), p)
                    accs[u, j] = o if n == 0 else accs[u, j] + o
                    if n == last:
                        o, b = _normalise(accs.pop((u, j)), u % 2)
                        rows = pl.ds(pl.multiple_of((A_HEADS * it + u) * HP, HP), HP)
                        OT[rows, pl.ds(j * A_QUERIES, A_QUERIES)] = o
                        b = functools.reduce(jnp.maximum, [b[:, 128 * t:128 * (t + 1)] for t in range(tq)])
                        bad = b if bad is None else jnp.maximum(bad, b)
            bad = pacer.finish(pacer.now + 600, bad)
            BAD[...] = jnp.maximum(BAD[...], bad)
            return carry

        lax.fori_loop(0, H // A_HEADS, body, 0)

    def attention_a_shifted():
        def body(it, carry):
            pair, t = it // (S // 128), it % (S // 128)
            for odd in range(2):
                s = _dot(KA[odd], QT[2 * pair + odd, t])
                p = jnp.exp2(s - jnp.max(s, axis=0, keepdims=True)).astype(BF)
                o, _ = _normalise(_dot(_tiles(VA, (odd,), 0, S), p), odd)
                OT[pl.ds(pl.multiple_of((2 * pair + odd) * HP, HP), HP), pl.ds(pl.multiple_of(t * 128, 128), 128)] = o
            return carry

        lax.fori_loop(0, (H // 2) * (S // 128), body, 0)

    def window_probs(h, i, b0, shifted):
        row = lax.broadcasted_iota(jnp.int32, (32, 128), 0)
        lane = lax.broadcasted_iota(jnp.int32, (32, 128), 1)
        q = QT.bitcast(U32)[h, i]
        w = jnp.concatenate([jnp.where(lane[0:16] // 32 == g, q, jnp.uint32(0)) for g in range(4)], axis=0)
        k0 = 64 * i - 80 + 16 * b0
        if not isinstance(k0, int):
            k0 = pl.multiple_of(k0, 16)
        s = _dot(pltpu.bitcast(KS[h, pl.ds(k0, 16 * (9 - b0)), :], BF), pltpu.bitcast(w, BF))
        e = {b: s[32 * (b - b0):32 * (b - b0 + 1)] for b in range(b0, 9)}
        masked = -jnp.inf if shifted else 0.0
        if not shifted:
            e = {b: jnp.exp2(v) for b, v in e.items()}
        if b0 == 0:
            e[0] = jnp.where(row > lane % 32, e[0], masked)
        e[8] = jnp.where(row <= lane % 32, e[8], masked)
        if shifted:
            for b in range(b0, b0 + 3 if b0 else b0):
                e[b] = jnp.where(lane // 32 >= 3 - (b - b0), e[b], masked)
            m = jnp.max(functools.reduce(jnp.maximum, e.values()), axis=0, keepdims=True)
            e = {b: jnp.exp2(v - m) for b, v in e.items()}

        def pick(mask, a, b):
            if a is None and b is None:
                return None
            return jnp.where(mask, 0.0 if a is None else a, 0.0 if b is None else b)

        f = {b: pick((lane // 32) % 2 == 1, e.get(b - 1), e.get(b)) for b in range(10)}
        start = {5: 8, 1: 4, 0: 0}[b0]
        p = [pick(lane >= 64, f.get(b - 2), f.get(b)) for b in range(start, 12)]
        return jnp.concatenate(p, axis=0).astype(BF)

    def window_output(h, odd, i, p):
        v = jnp.concatenate([_words(VB, (h, i - t)) for t in reversed(range(p.shape[0] // 128))], axis=1)
        o, bad = _normalise(_dot(v, p), odd)
        r0 = h * HP if isinstance(h, int) else pl.multiple_of(h * HP, HP)
        q0 = 128 * i if isinstance(i, int) else pl.multiple_of(128 * i, 128)
        OT[pl.ds(r0, HP), pl.ds(q0, 128)] = o
        return bad

    def attention_b():
        @pl.when(ZERO[15] == 0)
        def _():
            items = [(i, h) for i in range(S // 128) for h in range(H)]
            bad = None
            for n in range(len(items) + B_LAG):
                if n < len(items):
                    i, h = items[n]
                    p = window_probs(h, i, max(0, 5 - 4 * i), False)
                    PB[n % B_SLOTS][ZERO[0], pl.ds(0, p.shape[0]), :] = p
                if n >= B_LAG:
                    i, h = items[n - B_LAG]
                    p = _words(PB[(n - B_LAG) % B_SLOTS], (0, pl.ds(0, 64 * min(i + 1, 3))))
                    b = window_output(h, h % 2, i, p)
                    bad = b if bad is None else jnp.maximum(bad, b)
            BAD[...] = jnp.maximum(BAD[...], bad)

    def attention_b_shifted():
        def body(pair, carry):
            for odd in range(2):
                h = 2 * pair + odd
                window_output(h, odd, 0, window_probs(h, 0, 5, True))
                window_output(h, odd, 1, window_probs(h, 1, 1, True))

                def inner(i, c):
                    window_output(h, odd, i, window_probs(h, i, 0, True))
                    return c

                lax.fori_loop(2, S // 128, inner, 0)
            return carry

        lax.fori_loop(0, H // 2, body, 0)

    def guarded(plain, shifted):
        BAD[...] = jnp.zeros(BAD.shape, F32)
        plain()

        @pl.when(jnp.max(BAD[...]) > 0.0)
        def _():
            shifted()

    x_copies = [pltpu.make_async_copy(xT_hbm.at[:, pl.ds(c * TC, TC)], x_io.at[:, pl.ds(c * TC, TC)], sems.at[c])
                for c in range(NCH)]
    w_copies = [pltpu.make_async_copy(src, dst, sems.at[NCH + i]) for i, (src, dst) in enumerate([
        (wq_hbm, wq_in), (wkT_hbm, wkT_in), (wvT_hbm, wvT_in),
        (woa_hbm, woa_in), (wqkv_hbm, wqkv_in), (wob_hbm, wob_in)])]
    for cp in w_copies[:3] + x_copies:
        cp.start()
    for i in range(16):
        ZERO[i] = 0
    PACE[ZERO[0] + 1] = jnp.zeros((8, 128), F32)
    for vp in VP:
        vp[A_QUERIES // 128, pl.ds(0, 16), :] = jnp.zeros((16, 128), BF)

    def io_quadrant(chunk, i, j):
        return pl.ds(i * HALF, HALF), pl.ds(128 * half_tiles(chunk, j)[0], TC // 2)

    def first_projection(chunk):
        for j in range(2):
            for i in range(2):
                put_x(chunk, i, j, x_io[io_quadrant(chunk, i, j)].astype(F32))
        project_a(chunk, layernorm(chunk))

    for cp in w_copies[:3]:
        cp.wait()
    wt = wq_in[...].T.astype(F32) * QSCALE
    pad = jnp.zeros((HP - DH, D), F32)
    _put_weight(WA, jnp.concatenate([wkT_in[...].astype(F32), pad, wt[:HALF]], axis=0),
                jnp.concatenate([wvT_in[...].astype(F32), pad, wt[HALF:]], axis=0))
    x_copies[0].wait()
    first_projection(chunks(TC)[0])
    for cp in x_copies[1:]:
        cp.wait()
    for cp in w_copies[3:]:
        cp.start()
    for chunk in chunks(TC)[1:]:
        first_projection(chunk)

    for layer_pair in range(2):
        guarded(attention_a, attention_a_shifted)
        if layer_pair == 0:
            for cp in w_copies[3:]:
                cp.wait()
            put_wo(woa_in, WOA)
            wt = wqkv_in[...].T.astype(F32)
            for pos, w in enumerate((wt[D:2 * D], wt[0:D] * QSCALE, wt[2 * D:3 * D])):
                _put_weight(WB, w[:HALF], w[HALF:], pos * HALF)
        k_prev = [jnp.zeros((48, H * HP // 2), U32)] * 2
        between_layers(WOA, functools.partial(project_b, k_prev=k_prev), TC if layer_pair else 2 * TC)
        if layer_pair == 0:
            put_wo(wob_in, WOB)
        guarded(attention_b, attention_b_shifted)
        if layer_pair == 0:
            between_layers(WOB, project_a, TC, 7 * (HALF + HP))

    outs = []

    def send(idx):
        outs.append(pltpu.make_async_copy(x_io.at[idx], out_hbm.at[idx], sems.at[len(outs)]))
        outs[-1].start()

    def emit(chunk, i, j, x):
        x_io[io_quadrant(chunk, i, j)] = x.astype(BF)
        if chunk[-1] == S // 128 - 1:
            send(io_quadrant(chunk, i, j))

    for c, chunk in enumerate(chunks(TC)):
        out_proj(WOB, chunk, emit)
        if c < NCH - 1:
            send((slice(None), pl.ds(c * TC, TC)))
    for cp in outs:
        cp.wait()


@jax.jit
def pallas_interleave_layers__grouped_kv_mqa__sliding_block__prompt_kernel(
    A_x: jax.Array,
    A_wq: jax.Array,
    A_wk: jax.Array,
    A_wv: jax.Array,
    A_wo: jax.Array,
    B_x: jax.Array,
    B_wqkv: jax.Array,
    B_wo: jax.Array,
):
    del B_x

    def weight(n):
        return pltpu.VMEM((7, 2, n, 128), BF)

    hbm = pl.BlockSpec(memory_space=pl.ANY)
    tq = A_QUERIES // 128
    out_t = pl.pallas_call(
        _kernel,
        out_shape=jax.ShapeDtypeStruct((D, S), BF),
        in_specs=[hbm] * 7,
        out_specs=hbm,
        scratch_shapes=[
            pltpu.VMEM((D, S), BF),
            pltpu.VMEM((D, D), BF), pltpu.VMEM((DH, D), BF), pltpu.VMEM((DH, D), BF),
            pltpu.VMEM((D, D), BF), pltpu.VMEM((D, 3 * D), BF), pltpu.VMEM((D, D), BF),
            weight(HALF + HP), weight(HALF), weight(3 * HALF), weight(HALF),
            pltpu.VMEM((H, S // 128, HP, 128), BF),
            pltpu.VMEM((H, HP, S), F32),
            pltpu.VMEM((2, S, HP), BF),
            pltpu.VMEM((HP, 256), F32),
            pltpu.VMEM((DH * VPU_KEYS, 128), F32),
            pltpu.VMEM((2, S // 128, HP, 128), BF),
            pltpu.VMEM((H, S // 2, 128), U32),
            pltpu.VMEM((H, S // 128, HP, 128), BF),
            pltpu.VMEM((H * HP, S), F32),
            pltpu.VMEM((8, 128), F32),
            pltpu.VMEM((3, 8, 128), F32),
            pltpu.SMEM((16,), jnp.int32),
            pltpu.SemaphoreType.DMA((16,)),
            [pltpu.VMEM((TC // 128, D, 128), F32)] * NCH,
            [pltpu.VMEM((tq + 1, VPU_KEYS, 128), BF)] * (A_HEADS * (S // A_QUERIES)),
            [pltpu.VMEM((tq, A_KEYS, 128), BF)] * A_SLOTS,
            [pltpu.VMEM((1, 384, 128), BF)] * B_SLOTS,
        ],
        compiler_params=pltpu.CompilerParams(vmem_limit_bytes=100 * 1024 * 1024),
        name="interleaved_attention",
    )(A_x.reshape(S, D).T, A_wq, A_wk.T, A_wv.T, A_wo, B_wqkv, B_wo)
    return out_t.T.reshape(1, S, D)
```

```python
import functools

import jax
import jax.numpy as jnp
import numpy as np
from jax import lax
import jax.experimental.pallas as pl
import jax.experimental.pallas.tpu as pltpu

BF = jnp.bfloat16
F32 = jnp.float32
U32 = jnp.uint32

S = 2048
D = 448
H = 16
DH = D // H
HP = 32
HALF = D // 2
EPS = 1e-5
QSCALE = float(DH ** -0.5 * np.log2(np.e))

L_MIN = 2.0 ** -30
ACC_MAX = 2.0 ** 100

TC = 512
NCH = S // TC

A_KEYS = 256
A_QUERIES = 128
A_HEADS = 2
A_LAG = 16
A_SLOTS = 32
VPU_KEYS = 224
VPU_PERIOD = 36
VPU_SLACK = 2750
B_LAG = 16
B_SLOTS = 32


def _dot(a, b):
    return lax.dot_general(a, b, (((1,), (0,)), ((), ())), preferred_element_type=F32)


def _words(ref, idx):
    return pltpu.bitcast(ref.bitcast(U32)[idx], BF)


def _tiles(ref, pre, c0, n):
    return jnp.concatenate([_words(ref, pre + (t,)) for t in range(c0 // 128, (c0 + n) // 128)], axis=1)


def _put_tiles(ref, pre, c0, val):
    for t in range(val.shape[1] // 128):
        ref[pre + (c0 // 128 + t,)] = val[:, 128 * t:128 * (t + 1)].astype(BF)


def _pad_head(rows, h, fill):
    r0 = 2 * DH * (h // 2) + (2 * DH - HP if h % 2 else 0)
    w = rows[r0:r0 + HP]
    if fill is None:
        return w
    sub = lax.broadcasted_iota(jnp.int32, (8, rows.shape[1]), 0)
    if h % 2 == 0:
        return jnp.concatenate([w[0:24], jnp.where(sub < 4, w[24:32], fill)], axis=0)
    return jnp.concatenate([jnp.where(sub >= 4, w[0:8], fill), w[8:32]], axis=0)


def _normalise(acc, odd):
    l = acc[0:1] if odd else acc[HP - 1:HP]
    o = acc * (1.0 / l)
    mag = jnp.max(jnp.abs(acc).reshape(HP // 8, 8, acc.shape[1]), axis=0)
    return o, jnp.where((mag <= ACC_MAX) & (l >= L_MIN), 0.0, 1.0)


def _put_weight(dst, top, bottom, r0=0):
    k = top.shape[1] // 2
    a11, a12, a21, a22 = top[:, :k], top[:, k:], bottom[:, :k], bottom[:, k:]
    for i, a in enumerate([a11 + a22, a21 + a22, a11, a22, a11 + a12, a21 - a11, a12 - a22]):
        for t in range(2):
            k1 = min(128 * (t + 1), k)
            dst[i, t, pl.ds(r0, a.shape[0]), pl.ds(0, k1 - 128 * t)] = a[:, 128 * t:k1].astype(BF)


def _matmul(w, k, rhs, done):
    def product(i, b):
        lhs = jnp.concatenate([_words(w, (i, 0)), _words(w, (i, 1, slice(None), slice(0, k - 128)))], axis=1)
        return _dot(lhs, b.astype(BF))

    b11, b12, b21, b22 = (0, 1), (0, 0), (1, 1), (1, 0)
    m2 = product(1, rhs(b11))
    m5 = product(4, rhs(b22))
    m1 = product(0, rhs(b11, b22))
    c11, c22 = m1 - m5, m1 - m2
    m3 = product(2, rhs(b12, b22, True))
    done(0, 0, m3 + m5)
    c22 = c22 + m3
    done(1, 0, c22 + product(5, rhs(b11, b12)))
    m4 = product(3, rhs(b21, b11, True))
    done(1, 1, m2 + m4)
    c11 = c11 + m4
    done(0, 1, c11 + product(6, rhs(b21, b22)))


class _Pacer:
    def __init__(self, scratch):
        self.scratch = scratch
        self.never = scratch[1] != 0.0
        self.tick = jnp.ones((8, 128), F32)
        self.clock = self.now = None

    def advance(self, cycle):
        while self.clock is not None and self.now + 2 <= cycle:
            self.clock, self.now = self.clock + self.tick, self.now + 2

    def mark(self, cycle, value):
        self.advance(cycle)
        if self.clock is None:
            self.clock, self.now = value, cycle
        else:
            self.clock, self.now = jnp.where(self.never, value, self.clock), self.now + 1

    def finish(self, cycle, result):
        self.advance(cycle)
        self.scratch[0] = jnp.zeros((8, 128), F32)
        return jnp.where(self.scratch[0] != 0.0, self.clock, result)


def _kernel(xT_hbm, wq_hbm, wkT_hbm, wvT_hbm, woa_hbm, wqkv_hbm, wob_hbm, out_hbm,
            x_io, wq_in, wkT_in, wvT_in, woa_in, wqkv_in, wob_in,
            WA, WOA, WB, WOB, QT, QF, KA, KF, KBC, VA, KS, VB, OT, BAD, PACE, ZERO, sems,
            X, VP, PA, PB):

    def half_tiles(chunk, j):
        n = len(chunk) // 2
        return chunk[j * n:(j + 1) * n]

    def x_tile(base, t, i):
        return X[t // 4], (base + t % 4, pl.ds(i * HALF, HALF))

    def put_x(chunk, i, j, x):
        for n, t in enumerate(half_tiles(chunk, j)):
            ref, idx = x_tile(ZERO[0], t, i)
            ref[idx] = x[:, 128 * n:128 * (n + 1)]

    def get_x(base, t, i):
        ref, idx = x_tile(base, t, i)
        return ref[idx]

    def layernorm(chunk, pacer=None, now=0):
        def mean_of(v):
            part = jnp.sum(v.reshape(D // 32, 32, 128), axis=0)
            return jnp.sum(part, axis=0, keepdims=True) * (1.0 / D)

        coef, calls = {}, [0]
        for n, t in enumerate(chunk):
            x = X[t // 4][t % 4]
            mean = mean_of(x)
            centred = x - mean
            inv = lax.rsqrt(mean_of(centred * centred) + EPS)
            coef[t] = (inv, mean * inv)
            if pacer is not None:
                pacer.mark(now + 300 + 200 * n, jnp.broadcast_to(inv, (8, 128)))

        def quadrant(p, q=None, minus=False):
            calls[0] += 1
            base, out = ZERO[calls[0]], []
            for t, u in zip(half_tiles(chunk, p[1]), half_tiles(chunk, (q or p)[1])):
                if q is None:
                    out.append(get_x(base, t, p[0]) * coef[t][0] - coef[t][1])
                elif minus:
                    out.append((get_x(base, t, p[0]) - get_x(base, u, q[0])) * coef[t][0])
                else:
                    out.append(get_x(base, t, p[0]) * coef[t][0] + get_x(base, u, q[0]) * coef[u][0]
                               - (coef[t][1] + coef[u][1]))
            return jnp.concatenate(out, axis=1)

        return quadrant

    def project_a(chunk, xn):
        def done(i, j, r):
            c0 = 128 * half_tiles(chunk, j)[0]
            cols = pl.ds(c0, r.shape[1])
            q = r[HP:]
            for h in range(H // 2):
                qh = _pad_head(q, h, None)
                _put_tiles(QT, (h + i * (H // 2),), c0, qh)
                QF[h + i * (H // 2), :, cols] = qh
            even = r[0:HP]
            odd = jnp.concatenate([even[DH:HP], even[0:DH]], axis=0)
            sub = lax.broadcasted_iota(jnp.int32, even.shape, 0)
            spare = 0.0 if i == 0 else 1.0
            even, odd = jnp.where(sub < DH, even, spare), jnp.where(sub >= HP - DH, odd, spare)
            if i == 0:
                KA[0, cols, :] = even.astype(BF).T
                KA[1, cols, :] = odd.astype(BF).T
                if c0 == 0:
                    KF[...] = even[:, 0:256]
                if c0 == TC:
                    kt = KF[...].T[0:VPU_KEYS]
                    for d in range(DH):
                        KBC[pl.ds(d * VPU_KEYS, VPU_KEYS), :] = jnp.broadcast_to(kt[:, d:d + 1], (VPU_KEYS, 128))
            else:
                _put_tiles(VA, (0,), c0, even)
                _put_tiles(VA, (1,), c0, odd)

        _matmul(WA, HALF, xn, done)

    def project_b(chunk, xn, k_prev):
        def done(i, j, r):
            c0 = 128 * half_tiles(chunk, j)[0]
            k, q, v = r[0:HALF], r[HALF:2 * HALF], r[2 * HALF:3 * HALF]
            kp = jnp.concatenate([_pad_head(k, h, 0.0) for h in range(H // 2)], axis=0)
            kt = pltpu.bitcast(kp.astype(BF).T, U32)
            ext = jnp.concatenate([k_prev[i], kt], axis=0)
            n = kt.shape[0]
            k_prev[i] = kt[n - 48:]
            group = lax.broadcasted_iota(jnp.int32, (n, 128), 1) >> 5
            is_group = [group == g for g in range(4)]
            for h0 in range(0, H // 2, 4):
                four = ext[:, HP * h0:HP * (h0 + 4)]
                rolled = [four] + [pltpu.roll(four, HP * s, 1) for s in (1, 2, 3)]
                for h in range(4):
                    w = rolled[-h % 4][0:n]
                    for g in (1, 2, 3):
                        w = jnp.where(is_group[g], rolled[(g - h) % 4][16 * g:16 * g + n], w)
                    KS[h0 + h + i * (H // 2), pl.ds(c0 // 2, n), :] = w
            for h in range(H // 2):
                _put_tiles(QT, (h + i * (H // 2),), c0, _pad_head(q, h, None))
                _put_tiles(VB, (h + i * (H // 2),), c0, _pad_head(v, h, 1.0))

        _matmul(WB, HALF, xn, done)

    def out_proj(wo, chunk, done):
        def load(i, j):
            tiles = half_tiles(chunk, j)
            return OT[pl.ds(i * 256, 256), pl.ds(128 * tiles[0], 128 * len(tiles))]

        def quadrant(p, q=None, minus=False):
            return load(*p) if q is None else load(*p) - load(*q) if minus else load(*p) + load(*q)

        def add_residual(i, j, r):
            done(chunk, i, j, jnp.concatenate([get_x(0, t, i) for t in half_tiles(chunk, j)], axis=1) + r)

        _matmul(wo, 256, quadrant, add_residual)

    def chunks(tokens):
        return [range(t, t + tokens // 128) for t in range(0, S // 128, tokens // 128)]

    def between_layers(wo, project, tokens, cycles=None):
        parts = chunks(tokens)
        out_proj(wo, parts[0], put_x)
        now, xn = 7 * HALF, {}
        pacer = _Pacer(PACE) if cycles else None
        for c, chunk in enumerate(parts):
            if c not in xn:
                xn[c] = layernorm(chunk, pacer, now)
            if c + 1 < len(parts):
                out_proj(wo, parts[c + 1], put_x)
                now += 7 * HALF
            if c + 2 == len(parts):
                xn[c + 1] = layernorm(parts[c + 1], pacer, now)
            project(chunk, xn[c])
            now += cycles or 0
        if cycles:
            PACE[2] = pacer.finish(now + 200, jnp.zeros((8, 128), F32))

    def put_wo(src, dst):
        w = src[...].astype(F32)
        wt = jnp.concatenate([_pad_head(w, h, 0.0) for h in range(H)], axis=0).astype(BF).T.astype(F32)
        _put_weight(dst, wt[:HALF], wt[HALF:])

    def attention_a():
        first = -(-VPU_KEYS // A_KEYS) * A_KEYS
        ranges = [(k0, k0 + A_KEYS) for k0 in range(first, S, A_KEYS)] + [(VPU_KEYS, first)]
        last = len(ranges) - 1
        n_q, tq = S // A_QUERIES, A_QUERIES // 128

        def body(it, carry):
            zero = ZERO[0]
            pacer = _Pacer(PACE)

            def vpu_probs():
                j = 0
                for u in range(A_HEADS):
                    qf = QF.at[A_HEADS * it + u]
                    for t in range(S // 128):
                        vp, q = VP[u * n_q + t // tq], {}
                        for r in range(0, VPU_KEYS, 16):
                            s = None
                            for d in range(DH):
                                if d not in q:
                                    row = qf[pl.ds(d + 4 * (u % 2), 1), pl.ds(t * 128, 128)]
                                    q[d] = jnp.broadcast_to(row, (16, 128))
                                term = KBC[pl.ds(d * VPU_KEYS + r, 16), :] * q[d]
                                s = term if s is None else s + term
                            vp[zero + t % tq, pl.ds(r, 16), :] = jnp.exp2(s).astype(BF)
                            pacer.mark(j * VPU_PERIOD, vp.bitcast(F32)[tq, pl.ds(0, 8), :])
                            j += 1
                            pacer.advance(j * VPU_PERIOD)

            items = [(u, n, j) for u in range(A_HEADS) for n in range(last) for j in range(n_q)]
            n_plain = len(items)
            items += [(u, last, j) for u in range(A_HEADS) for j in range(n_q)]
            accs, bad = {}, None
            for i in range(len(items) + A_LAG):
                if i == n_plain:
                    vpu_probs()
                if i < len(items):
                    u, n, j = items[i]
                    k0, k1 = ranges[n]
                    k = _words(KA, (u % 2, pl.ds(k0 // 2, (k1 - k0) // 2)))
                    p = jnp.exp2(_dot(k, _tiles(QT, (A_HEADS * it + u,), j * A_QUERIES, A_QUERIES)))
                    for t in range(tq):
                        PA[i % A_SLOTS][zero + t, pl.ds(0, k1 - k0), :] = p[:, 128 * t:128 * (t + 1)].astype(BF)
                if i >= A_LAG:
                    u, n, j = items[i - A_LAG]
                    k0, k1 = ranges[n]
                    slot = PA[(i - A_LAG) % A_SLOTS]
                    p = jnp.concatenate([_words(slot, (t, pl.ds(0, (k1 - k0) // 2))) for t in range(tq)], axis=1)
                    if n == last:
                        p = jnp.concatenate([_tiles(VP[u * n_q + j], (), 0, A_QUERIES), p], axis=0)
                        k0 = 0
                    o = _dot(_tiles(VA, (u % 2,), k0, k1 - k0), p)
                    accs[u, j] = o if n == 0 else accs[u, j] + o
                    if n == last:
                        o, b = _normalise(accs.pop((u, j)), u % 2)
                        rows = pl.ds(pl.multiple_of((A_HEADS * it + u) * HP, HP), HP)
                        OT[rows, pl.ds(j * A_QUERIES, A_QUERIES)] = o
                        b = functools.reduce(jnp.maximum, [b[:, 128 * t:128 * (t + 1)] for t in range(tq)])
                        bad = b if bad is None else jnp.maximum(bad, b)
            bad = pacer.finish(pacer.now + VPU_SLACK, bad)
            BAD[...] = jnp.maximum(BAD[...], bad)
            return carry

        lax.fori_loop(0, H // A_HEADS, body, 0)

    def attention_a_shifted():
        def body(it, carry):
            pair, t = it // (S // 128), it % (S // 128)
            for odd in range(2):
                s = _dot(KA[odd], QT[2 * pair + odd, t])
                p = jnp.exp2(s - jnp.max(s, axis=0, keepdims=True)).astype(BF)
                o, _ = _normalise(_dot(_tiles(VA, (odd,), 0, S), p), odd)
                OT[pl.ds(pl.multiple_of((2 * pair + odd) * HP, HP), HP), pl.ds(pl.multiple_of(t * 128, 128), 128)] = o
            return carry

        lax.fori_loop(0, (H // 2) * (S // 128), body, 0)

    def window_masks():
        row = lax.broadcasted_iota(jnp.int32, (32, 128), 0)
        lane = lax.broadcasted_iota(jnp.int32, (32, 128), 1)
        group, query = lane >> 5, lane & 31
        return dict(group=group, own=[group[0:16] == g for g in range(4)], no_word=jnp.zeros((16, 128), U32),
                    oldest=row > query, newest=row <= query, odd=(group & 1) == 1, high=group >= 2,
                    zero=jnp.zeros((32, 128), F32))

    def window_probs(h, i, b0, masks, shifted):
        q = QT.bitcast(U32)[h, i]
        w = jnp.concatenate([jnp.where(own, q, masks["no_word"]) for own in masks["own"]], axis=0)
        k0 = 64 * i - 80 + 16 * b0
        if not isinstance(k0, int):
            k0 = pl.multiple_of(k0, 16)
        s = _dot(pltpu.bitcast(KS[h, pl.ds(k0, 16 * (9 - b0)), :], BF), pltpu.bitcast(w, BF))
        if not shifted:
            s = jnp.exp2(s)
        e = {b: s[32 * (b - b0):32 * (b - b0 + 1)] for b in range(b0, 9)}
        masked = -jnp.inf if shifted else masks["zero"]
        if b0 == 0:
            e[0] = jnp.where(masks["oldest"], e[0], masked)
        e[8] = jnp.where(masks["newest"], e[8], masked)
        if shifted:
            for b in range(b0, b0 + 3 if b0 else b0):
                e[b] = jnp.where(masks["group"] >= 3 - (b - b0), e[b], masked)
            m = jnp.max(functools.reduce(jnp.maximum, e.values()), axis=0, keepdims=True)
            e = {b: jnp.exp2(v - m) for b, v in e.items()}

        def pick(mask, a, b):
            if a is None and b is None:
                return None
            return jnp.where(mask, masks["zero"] if a is None else a, masks["zero"] if b is None else b)

        f = {b: pick(masks["odd"], e.get(b - 1), e.get(b)) for b in range(10)}
        start = {5: 8, 1: 4, 0: 0}[b0]
        p = [pick(masks["high"], f.get(b - 2), f.get(b)) for b in range(start, 12)]
        return jnp.concatenate(p, axis=0).astype(BF)

    def window_output(h, odd, i, p):
        v = jnp.concatenate([_words(VB, (h, i - t)) for t in reversed(range(p.shape[0] // 128))], axis=1)
        o, bad = _normalise(_dot(v, p), odd)
        r0 = h * HP if isinstance(h, int) else pl.multiple_of(h * HP, HP)
        q0 = 128 * i if isinstance(i, int) else pl.multiple_of(128 * i, 128)
        OT[pl.ds(r0, HP), pl.ds(q0, 128)] = o
        return bad

    def attention_b():
        @pl.when(ZERO[15] == 0)
        def _():
            items = [(i, h) for i in range(S // 128) for h in range(H)]
            masks, bad = window_masks(), None
            for n in range(len(items) + B_LAG):
                if n < len(items):
                    i, h = items[n]
                    p = window_probs(h, i, max(0, 5 - 4 * i), masks, False)
                    PB[n % B_SLOTS][ZERO[0], pl.ds(0, p.shape[0]), :] = p
                if n >= B_LAG:
                    i, h = items[n - B_LAG]
                    p = _words(PB[(n - B_LAG) % B_SLOTS], (0, pl.ds(0, 64 * min(i + 1, 3))))
                    b = window_output(h, h % 2, i, p)
                    bad = b if bad is None else jnp.maximum(bad, b)
            BAD[...] = jnp.maximum(BAD[...], bad)

    def attention_b_shifted():
        def body(pair, carry):
            for odd in range(2):
                h = 2 * pair + odd
                window_output(h, odd, 0, window_probs(h, 0, 5, window_masks(), True))
                window_output(h, odd, 1, window_probs(h, 1, 1, window_masks(), True))

                def inner(i, c):
                    window_output(h, odd, i, window_probs(h, i, 0, window_masks(), True))
                    return c

                lax.fori_loop(2, S // 128, inner, 0)
            return carry

        lax.fori_loop(0, H // 2, body, 0)

    def guarded(plain, shifted):
        BAD[...] = jnp.zeros(BAD.shape, F32)
        plain()

        @pl.when(jnp.max(BAD[...]) > 0.0)
        def _():
            shifted()

    x_copies = [pltpu.make_async_copy(xT_hbm.at[:, pl.ds(c * TC, TC)], x_io.at[:, pl.ds(c * TC, TC)], sems.at[c])
                for c in range(NCH)]
    w_copies = [pltpu.make_async_copy(src, dst, sems.at[NCH + i]) for i, (src, dst) in enumerate([
        (wq_hbm, wq_in), (wkT_hbm, wkT_in), (wvT_hbm, wvT_in),
        (woa_hbm, woa_in), (wqkv_hbm, wqkv_in), (wob_hbm, wob_in)])]
    for cp in w_copies[:3] + x_copies:
        cp.start()
    for i in range(16):
        ZERO[i] = 0
    PACE[ZERO[0] + 1] = jnp.zeros((8, 128), F32)
    for vp in VP:
        vp[A_QUERIES // 128, pl.ds(0, 16), :] = jnp.zeros((16, 128), BF)

    def io_quadrant(chunk, i, j):
        return pl.ds(i * HALF, HALF), pl.ds(128 * half_tiles(chunk, j)[0], TC // 2)

    def first_projection(chunk):
        for j in range(2):
            for i in range(2):
                put_x(chunk, i, j, x_io[io_quadrant(chunk, i, j)].astype(F32))
        project_a(chunk, layernorm(chunk))

    for cp in w_copies[:3]:
        cp.wait()
    wt = wq_in[...].T.astype(F32) * QSCALE
    pad = jnp.zeros((HP - DH, D), F32)
    _put_weight(WA, jnp.concatenate([wkT_in[...].astype(F32), pad, wt[:HALF]], axis=0),
                jnp.concatenate([wvT_in[...].astype(F32), pad, wt[HALF:]], axis=0))
    x_copies[0].wait()
    first_projection(chunks(TC)[0])
    for cp in x_copies[1:]:
        cp.wait()
    for cp in w_copies[3:]:
        cp.start()
    for chunk in chunks(TC)[1:]:
        first_projection(chunk)

    for layer_pair in range(2):
        guarded(attention_a, attention_a_shifted)
        if layer_pair == 0:
            for cp in w_copies[3:]:
                cp.wait()
            put_wo(woa_in, WOA)
            wt = wqkv_in[...].T.astype(F32)
            for pos, w in enumerate((wt[D:2 * D], wt[0:D] * QSCALE, wt[2 * D:3 * D])):
                _put_weight(WB, w[:HALF], w[HALF:], pos * HALF)
        k_prev = [jnp.zeros((48, H * HP // 2), U32)] * 2
        between_layers(WOA, functools.partial(project_b, k_prev=k_prev), TC if layer_pair else 2 * TC)
        if layer_pair == 0:
            put_wo(wob_in, WOB)
        guarded(attention_b, attention_b_shifted)
        if layer_pair == 0:
            between_layers(WOB, project_a, TC, 7 * (HALF + HP))

    outs = []

    def send(idx):
        outs.append(pltpu.make_async_copy(x_io.at[idx], out_hbm.at[idx], sems.at[len(outs)]))
        outs[-1].start()

    def emit(chunk, i, j, x):
        x_io[io_quadrant(chunk, i, j)] = x.astype(BF)
        if chunk[-1] == S // 128 - 1:
            send(io_quadrant(chunk, i, j))

    for c, chunk in enumerate(chunks(TC)):
        out_proj(WOB, chunk, emit)
        if c < NCH - 1:
            send((slice(None), pl.ds(c * TC, TC)))
    for cp in outs:
        cp.wait()


@jax.jit
def pallas_interleave_layers__grouped_kv_mqa__sliding_block__prompt_kernel(
    A_x: jax.Array,
    A_wq: jax.Array,
    A_wk: jax.Array,
    A_wv: jax.Array,
    A_wo: jax.Array,
    B_x: jax.Array,
    B_wqkv: jax.Array,
    B_wo: jax.Array,
):
    del B_x

    def weight(n):
        return pltpu.VMEM((7, 2, n, 128), BF)

    hbm = pl.BlockSpec(memory_space=pl.ANY)
    tq = A_QUERIES // 128
    out_t = pl.pallas_call(
        _kernel,
        out_shape=jax.ShapeDtypeStruct((D, S), BF),
        in_specs=[hbm] * 7,
        out_specs=hbm,
        scratch_shapes=[
            pltpu.VMEM((D, S), BF),
            pltpu.VMEM((D, D), BF), pltpu.VMEM((DH, D), BF), pltpu.VMEM((DH, D), BF),
            pltpu.VMEM((D, D), BF), pltpu.VMEM((D, 3 * D), BF), pltpu.VMEM((D, D), BF),
            weight(HALF + HP), weight(HALF), weight(3 * HALF), weight(HALF),
            pltpu.VMEM((H, S // 128, HP, 128), BF),
            pltpu.VMEM((H, HP, S), F32),
            pltpu.VMEM((2, S, HP), BF),
            pltpu.VMEM((HP, 256), F32),
            pltpu.VMEM((DH * VPU_KEYS, 128), F32),
            pltpu.VMEM((2, S // 128, HP, 128), BF),
            pltpu.VMEM((H, S // 2, 128), U32),
            pltpu.VMEM((H, S // 128, HP, 128), BF),
            pltpu.VMEM((H * HP, S), F32),
            pltpu.VMEM((8, 128), F32),
            pltpu.VMEM((3, 8, 128), F32),
            pltpu.SMEM((16,), jnp.int32),
            pltpu.SemaphoreType.DMA((16,)),
            [pltpu.VMEM((TC // 128, D, 128), F32)] * NCH,
            [pltpu.VMEM((tq + 1, VPU_KEYS, 128), BF)] * (A_HEADS * (S // A_QUERIES)),
            [pltpu.VMEM((tq, A_KEYS, 128), BF)] * A_SLOTS,
            [pltpu.VMEM((1, 384, 128), BF)] * B_SLOTS,
        ],
        compiler_params=pltpu.CompilerParams(vmem_limit_bytes=100 * 1024 * 1024),
        name="interleaved_attention",
    )(A_x.reshape(S, D).T, A_wq, A_wk.T, A_wv.T, A_wo, B_wqkv, B_wo)
    return out_t.T.reshape(1, S, D)
```
